```python
import jax
import jax.numpy as jnp

def _softmax(x, axis=-1):
    return jax.nn.softmax(x, axis=axis)
def _gelu(x):
    return jax.nn.gelu(x, approximate=True)
def _silu(x):
    return jax.nn.silu(x)
def _sigmoid(x):
    return jax.nn.sigmoid(x)
def _layernorm(x, axis=-1, eps=1e-5):
    m = jnp.mean(x, axis=axis, keepdims=True)
    v = jnp.var(x, axis=axis, keepdims=True)
    return (x - m) / jnp.sqrt(v + eps)
def _scatter_add(tgt, idx, src, axis=0):
    return tgt.at[idx].add(src)
def _segment_sum(src, seg, n):
    return jax.ops.segment_sum(src, seg, n)
class _Rng:
    def __init__(self, key):
        self._k = key
    def _next(self):
        self._k, sub = jax.random.split(self._k)
        return sub
    def normal(self, shape):
        return jax.random.normal(self._next(), shape, dtype=jnp.bfloat16)
    def randint(self, lo, hi, shape):
        return jax.random.randint(self._next(), shape, lo, hi, dtype=jnp.int32)
    def uniform(self, shape, lo=0.0, hi=1.0):
        return jax.random.uniform(self._next(), shape, jnp.bfloat16, lo, hi)
    def permutation(self, n):
        return jax.random.permutation(self._next(), n)


kernel_name = 'concat_heads__gqa_block_cached__gqa_block_cached__near_ridge'

def setup_inputs():
    _rng = _Rng(jax.random.key(int.from_bytes(__import__("os").urandom(4), "little")))
    _w = (lambda a: (lambda t: t.astype(jnp.bfloat16) if jnp.issubdtype(t.dtype, jnp.floating) else t)(jnp.asarray(a)))
    def _A_setup():
        B, Sq, D = 8, 256, 640
        Hq, Hkv, Sk, Dh = 32, 32, 1024, 192
        assert Hq % Hkv == 0, (Hq, Hkv)
        return {
            "x": _w((lambda *s: _rng.normal(s) * 0.05)(B, Sq, D)),
            "k_cache": _w((lambda *s: _rng.normal(s) * 0.05)(B, Hkv, Sk, Dh)),
            "v_cache": _w((lambda *s: _rng.normal(s) * 0.05)(B, Hkv, Sk, Dh)),
            "wq": _w((lambda *s: _rng.normal(s) * 0.05)(D, Hq * Dh) * (D ** -0.5)),
            "wo": _w((lambda *s: _rng.normal(s) * 0.05)(Hq * Dh, D) * ((Hq * Dh) ** -0.5)),
        }
    _A_in = _A_setup()

    def _B_setup():
        B, Sq, D = 8, 256, 640
        Hq, Hkv, Sk, Dh = 32, 32, 1024, 192
        assert Hq % Hkv == 0, (Hq, Hkv)
        return {
            "x": _w((lambda *s: _rng.normal(s) * 0.05)(B, Sq, D)),
            "k_cache": _w((lambda *s: _rng.normal(s) * 0.05)(B, Hkv, Sk, Dh)),
            "v_cache": _w((lambda *s: _rng.normal(s) * 0.05)(B, Hkv, Sk, Dh)),
            "wq": _w((lambda *s: _rng.normal(s) * 0.05)(D, Hq * Dh) * (D ** -0.5)),
            "wo": _w((lambda *s: _rng.normal(s) * 0.05)(Hq * Dh, D) * ((Hq * Dh) ** -0.5)),
        }
    _B_in = _B_setup()

    return {
        "A_x": _A_in["x"],
        "A_k_cache": _A_in["k_cache"],
        "A_v_cache": _A_in["v_cache"],
        "A_wq": _A_in["wq"],
        "A_wo": _A_in["wo"],
        "B_x": _B_in["x"],
        "B_k_cache": _B_in["k_cache"],
        "B_v_cache": _B_in["v_cache"],
        "B_wq": _B_in["wq"],
        "B_wo": _B_in["wo"],
    }

def reference(A_x, A_k_cache, A_v_cache, A_wq, A_wo, B_x, B_k_cache, B_v_cache, B_wq, B_wo):
    def _A_ref(x, k_cache, v_cache, wq, wo):
        B, Sq, D = x.shape
        Hq, Dh = 32, 192
        Hkv = k_cache.shape[1]
        rep = Hq // Hkv
        q = (lambda x, *d: x.transpose(*d))((x @ wq).reshape(B, Sq, Hq, Dh), 0, 2, 1, 3)
        k = jnp.repeat(k_cache, rep, axis=1)
        v = jnp.repeat(v_cache, rep, axis=1)
        scores = jnp.einsum("bhqd,bhkd->bhqk", q, k) * (Dh ** -0.5)
        p = _softmax(scores, axis=-1)
        o = jnp.einsum("bhqk,bhkd->bhqd", p, v)
        return (lambda x, *d: x.transpose(*d))(o, 0, 2, 1, 3).reshape(B, Sq, Hq * Dh) @ wo

    def _B_ref(x, k_cache, v_cache, wq, wo):
        B, Sq, D = x.shape
        Hq, Dh = 32, 192
        Hkv = k_cache.shape[1]
        rep = Hq // Hkv
        q = (lambda x, *d: x.transpose(*d))((x @ wq).reshape(B, Sq, Hq, Dh), 0, 2, 1, 3)
        k = jnp.repeat(k_cache, rep, axis=1)
        v = jnp.repeat(v_cache, rep, axis=1)
        scores = jnp.einsum("bhqd,bhkd->bhqk", q, k) * (Dh ** -0.5)
        p = _softmax(scores, axis=-1)
        o = jnp.einsum("bhqk,bhkd->bhqd", p, v)
        return (lambda x, *d: x.transpose(*d))(o, 0, 2, 1, 3).reshape(B, Sq, Hq * Dh) @ wo

    a = _A_ref(A_x, A_k_cache, A_v_cache, A_wq, A_wo)
    b = _B_ref(B_x, B_k_cache, B_v_cache, B_wq, B_wo)
    return jnp.concatenate([a, b], axis=-1)
```

```python
import jax
import jax.numpy as jnp
from jax import lax
import jax.experimental.pallas as pl
import jax.experimental.pallas.tpu as pltpu

_LOG2E = 1.4426950408889634
_NT = (((1,), (1,)), ((), ()))
_ORDER = "Q0 Q1 S00 M00 S10 M10 P00 S01 M01 P10 S11 M11 P01 P11 O0 O1".split()


@jax.jit
def pallas_concat_heads__gqa_block_cached__gqa_block_cached__near_ridge_kernel(
    A_x: jax.Array,
    A_k_cache: jax.Array,
    A_v_cache: jax.Array,
    A_wq: jax.Array,
    A_wo: jax.Array,
    B_x: jax.Array,
    B_k_cache: jax.Array,
    B_v_cache: jax.Array,
    B_wq: jax.Array,
    B_wo: jax.Array,
):
    B, SQ, D = A_x.shape
    _, H, SK, DH = A_k_cache.shape
    NP = H // 2
    f32, bf16 = jnp.float32, jnp.bfloat16
    qscale = DH ** -0.5 * _LOG2E

    def kernel(ax, akt, avt, awq, awo, bx, bkt, bvt, bwq, bwo, out_ref, acc_ref, wot):
        p_id = pl.program_id(0)
        b = pl.program_id(1)
        xs, kts, vts, wqs = (ax, bx), (akt, bkt), (avt, bvt), (awq, bwq)

        @pl.when(b == 0)
        def _():
            wot[0] = awo[...].T
            wot[1] = bwo[...].T

        @pl.when(p_id == 0)
        def _():
            acc_ref[0, b] = jnp.zeros((D, SQ), f32)
            acc_ref[1, b] = jnp.zeros((D, SQ), f32)

        q, s, p, li, o = {}, {}, {}, {}, {}
        for op in _ORDER:
            k, br = op[0], int(op[1])
            h = int(op[2]) if len(op) > 2 else None
            if k == "Q":
                qq = jnp.dot(xs[br][b], wqs[br][...], preferred_element_type=f32)
                q[br] = (qq * qscale).astype(bf16)
            elif k == "S":
                s[br, h] = jnp.dot(q[br][:, h * DH:(h + 1) * DH],
                                   kts[br][h * DH:(h + 1) * DH, :],
                                   preferred_element_type=f32)
            elif k == "M":
                ss = s[br, h]
                m = jnp.max(ss, axis=-1, keepdims=True)
                e = jnp.exp2(ss - m)
                l = jnp.sum(e, axis=-1, keepdims=True)
                p[br, h] = e.astype(bf16)
                li[br, h] = jnp.transpose(jnp.broadcast_to(1.0 / l, (SQ, 128)))[0:1, :]
            elif k == "P":
                r = lax.dot_general(vts[br][h * DH:(h + 1) * DH, :], p[br, h], _NT,
                                    preferred_element_type=f32)
                o[br, h] = (r * li[br, h]).astype(bf16)
            elif k == "O":
                ot = jnp.concatenate([o[br, 0], o[br, 1]], axis=0)
                acc_ref[br, b] += jnp.dot(wot[br], ot, preferred_element_type=f32)

        @pl.when(p_id == NP - 1)
        def _():
            for br in range(2):
                out_ref[:, br * D:(br + 1) * D] = acc_ref[br, b].T.astype(bf16)

    def t(a):
        return jnp.swapaxes(a, 2, 3).reshape(B, NP, 2 * DH, SK)

    xs = pl.BlockSpec((B, SQ, D), lambda p, b: (0, 0, 0))
    kv = pl.BlockSpec((None, None, 2 * DH, SK), lambda p, b: (b, p, 0, 0))
    wq = pl.BlockSpec((D, 2 * DH), lambda p, b: (0, p))
    wo = pl.BlockSpec((2 * DH, D), lambda p, b: (p, 0))
    return pl.pallas_call(
        kernel,
        grid=(NP, B),
        in_specs=[xs, kv, kv, wq, wo] * 2,
        out_specs=pl.BlockSpec((None, SQ, 2 * D),
                               lambda p, b: (jnp.where(p == NP - 1, b, 0), 0, 0)),
        out_shape=jax.ShapeDtypeStruct((B, SQ, 2 * D), bf16),
        scratch_shapes=[pltpu.VMEM((2, B, D, SQ), f32), pltpu.VMEM((2, D, 2 * DH), bf16)],
        compiler_params=pltpu.CompilerParams(
            dimension_semantics=("arbitrary", "arbitrary"),
            vmem_limit_bytes=100 * 1024 * 1024),
    )(A_x, t(A_k_cache), t(A_v_cache), A_wq, A_wo,
      B_x, t(B_k_cache), t(B_v_cache), B_wq, B_wo)
```

```python
import jax
import jax.numpy as jnp
from jax import lax
import jax.experimental.pallas as pl
import jax.experimental.pallas.tpu as pltpu

_LOG2E = 1.4426950408889634
_NT = (((1,), (1,)), ((), ()))
_TN = (((0,), (0,)), ((), ()))
_NB = 2
_ORDER = ("Q0 Q1 S00 S01 P00 S10 P01 Q2 P10 Q3 S20 S11 O0 P11 "
          "S30 P20 S31 P30 S21 P31 O1 P21 O3 O2").split()


@jax.jit
def pallas_concat_heads__gqa_block_cached__gqa_block_cached__near_ridge_kernel(
    A_x: jax.Array,
    A_k_cache: jax.Array,
    A_v_cache: jax.Array,
    A_wq: jax.Array,
    A_wo: jax.Array,
    B_x: jax.Array,
    B_k_cache: jax.Array,
    B_v_cache: jax.Array,
    B_wq: jax.Array,
    B_wo: jax.Array,
):
    B, SQ, D = A_x.shape
    _, H, SK, DH = A_k_cache.shape
    NP, nb = H // 2, _NB
    NG = B // nb
    NI = NP * NG
    f32, bf16 = jnp.float32, jnp.bfloat16
    qscale = DH ** -0.5 * _LOG2E

    def kernel(ax, akt, avt, awq, awo, bx, bkt, bvt, bwq, bwo, out_hbm,
               x_v, k_v, v_v, wq_v, wo_v, acc_ref, o_v, sx, sk, sv, sq, so, sout):
        xh, kh, vh, wqh, woh = (ax, bx), (akt, bkt), (avt, bvt), (awq, bwq), (awo, bwo)

        def x_copy(g, br):
            return pltpu.make_async_copy(
                xh[br].at[pl.ds(g * nb, nb)], x_v.at[br, pl.ds(g * nb, nb)], sx.at[g * 2 + br])

        def kv_copy(src, dst, sem, i, br, bi):
            sl = i % 2
            return pltpu.make_async_copy(
                src[br].at[(i % NG) * nb + bi, i // NG], dst.at[sl, br, bi],
                sem.at[(sl * 2 + br) * nb + bi])

        def k_copy(i, br, bi):
            return kv_copy(kh, k_v, sk, i, br, bi)

        def v_copy(i, br, bi):
            return kv_copy(vh, v_v, sv, i, br, bi)

        def wq_copy(p, br):
            cols = pl.ds(pl.multiple_of(p * 2 * DH, 128), 2 * DH)
            return pltpu.make_async_copy(
                wqh[br].at[:, cols], wq_v.at[p % 2, br], sq.at[(p % 2) * 2 + br])

        def wo_copy(p, br):
            rows = pl.ds(pl.multiple_of(p * 2 * DH, 128), 2 * DH)
            return pltpu.make_async_copy(
                woh[br].at[rows, :], wo_v.at[p % 2, br], so.at[(p % 2) * 2 + br])

        def out_copy(g):
            return pltpu.make_async_copy(
                o_v.at[pl.ds(g * nb, nb)], out_hbm.at[pl.ds(g * nb, nb)], sout.at[g])

        for br in range(2):
            x_copy(0, br).start()
            wq_copy(0, br).start()
        for br in range(2):
            wo_copy(0, br).start()
        for bi in range(nb):
            for br in range(2):
                k_copy(0, br, bi).start()
            for br in range(2):
                v_copy(0, br, bi).start()
        for br in range(2):
            for b in range(B):
                acc_ref[br, b] = jnp.zeros((SQ, D), f32)

        def body(i, carry):
            p_id, g, sl = i // NG, i % NG, i % 2
            ws = p_id % 2

            todo = []
            for bi in range(nb):
                for cp in (k_copy, v_copy):
                    for br in range(2):
                        todo.append((i + 1 < NI, cp, (i + 1, br, bi)))
            for br in range(2):
                todo.append((i + 1 < NG, x_copy, (i + 1, br)))
            for cp in (wq_copy, wo_copy):
                for br in range(2):
                    todo.append((jnp.logical_and(g == 0, p_id + 1 < NP), cp, (p_id + 1, br)))

            @pl.when(i < NG)
            def _():
                for br in range(2):
                    x_copy(i, br).wait()

            @pl.when(g == 0)
            def _():
                for cp in (wq_copy, wo_copy):
                    for br in range(2):
                        cp(p_id, br).wait()

            q, p, linv, o = {}, {}, {}, {}
            for n, op in enumerate(_ORDER):
                if n >= 1 and todo:
                    cond, cp, args = todo.pop(0)
                    pl.when(cond)(lambda: cp(*args).start())
                kind, u = op[0], int(op[1])
                br, bi = u % 2, u // 2
                b = g * nb + bi
                if kind == "Q":
                    qq = jnp.dot(x_v[br, b], wq_v[ws, br], preferred_element_type=f32)
                    q[u] = (qq * qscale).astype(bf16)
                elif kind == "S":
                    h = int(op[2])
                    if h == 0:
                        k_copy(i, br, bi).wait()
                    s = jnp.dot(q[u][:, h * DH:(h + 1) * DH],
                                k_v[sl, br, bi, h * DH:(h + 1) * DH, :],
                                preferred_element_type=f32)
                    e = jnp.exp2(s - jnp.max(s, axis=-1, keepdims=True))
                    l = jnp.sum(e, axis=-1, keepdims=True)
                    p[u, h] = e.astype(bf16)
                    linv[u, h] = 1.0 / jnp.transpose(jnp.broadcast_to(l, (SQ, 128)))[0:1, :]
                elif kind == "P":
                    h = int(op[2])
                    if h == 0:
                        v_copy(i, br, bi).wait()
                    r = lax.dot_general(v_v[sl, br, bi, h * DH:(h + 1) * DH, :], p[u, h], _NT,
                                        preferred_element_type=f32)
                    o[u, h] = (r * linv[u, h]).astype(bf16)
                else:
                    ot = jnp.concatenate([o[u, 0], o[u, 1]], axis=0)
                    r = acc_ref[br, b] + lax.dot_general(
                        ot, wo_v[ws, br], _TN, preferred_element_type=f32)
                    acc_ref[br, b] = r
                    o_v[b, :, br * D:(br + 1) * D] = r.astype(bf16)

            @pl.when(p_id == NP - 1)
            def _():
                out_copy(g).start()
            return carry

        lax.fori_loop(0, NI, body, 0)
        for g in range(NG):
            out_copy(g).wait()

    def t(a):
        return jnp.swapaxes(a, 2, 3).reshape(B, NP, 2 * DH, SK)

    anyspec = pl.BlockSpec(memory_space=pl.ANY)
    return pl.pallas_call(
        kernel,
        in_specs=[anyspec] * 10,
        out_specs=anyspec,
        out_shape=jax.ShapeDtypeStruct((B, SQ, 2 * D), bf16),
        scratch_shapes=[
            pltpu.VMEM((2, B, SQ, D), bf16),
            pltpu.VMEM((2, 2, nb, 2 * DH, SK), bf16),
            pltpu.VMEM((2, 2, nb, 2 * DH, SK), bf16),
            pltpu.VMEM((2, 2, D, 2 * DH), bf16),
            pltpu.VMEM((2, 2, 2 * DH, D), bf16),
            pltpu.VMEM((2, B, SQ, D), f32),
            pltpu.VMEM((B, SQ, 2 * D), bf16),
            pltpu.SemaphoreType.DMA((2 * NG,)),
            pltpu.SemaphoreType.DMA((4 * nb,)),
            pltpu.SemaphoreType.DMA((4 * nb,)),
            pltpu.SemaphoreType.DMA((4,)),
            pltpu.SemaphoreType.DMA((4,)),
            pltpu.SemaphoreType.DMA((NG,)),
        ],
        compiler_params=pltpu.CompilerParams(
            vmem_limit_bytes=100 * 1024 * 1024,
            flags={"XLA_TPU_RESCHEDULE_DMA_DONES": True}),
    )(A_x, t(A_k_cache), t(A_v_cache), A_wq, A_wo,
      B_x, t(B_k_cache), t(B_v_cache), B_wq, B_wo)
```
